```python
import jax
import jax.numpy as jnp

def _softmax(x, axis=-1):
    return jax.nn.softmax(x, axis=axis)
def _gelu(x):
    return jax.nn.gelu(x, approximate=True)
def _silu(x):
    return jax.nn.silu(x)
def _sigmoid(x):
    return jax.nn.sigmoid(x)
def _layernorm(x, axis=-1, eps=1e-5):
    m = jnp.mean(x, axis=axis, keepdims=True)
    v = jnp.var(x, axis=axis, keepdims=True)
    return (x - m) / jnp.sqrt(v + eps)
def _scatter_add(tgt, idx, src, axis=0):
    return tgt.at[idx].add(src)
def _segment_sum(src, seg, n):
    return jax.ops.segment_sum(src, seg, n)
class _Rng:
    def __init__(self, key):
        self._k = key
    def _next(self):
        self._k, sub = jax.random.split(self._k)
        return sub
    def normal(self, shape):
        return jax.random.normal(self._next(), shape, dtype=jnp.bfloat16)
    def randint(self, lo, hi, shape):
        return jax.random.randint(self._next(), shape, lo, hi, dtype=jnp.int32)
    def uniform(self, shape, lo=0.0, hi=1.0):
        return jax.random.uniform(self._next(), shape, jnp.bfloat16, lo, hi)
    def permutation(self, n):
        return jax.random.permutation(self._next(), n)


kernel_name = 'recurrent_scan__compressed_kv_cla__dense_activation_silu__decode'

def setup_inputs():
    _rng = _Rng(jax.random.key(int.from_bytes(__import__("os").urandom(4), "little")))
    _w = (lambda a: (lambda t: t.astype(jnp.bfloat16) if jnp.issubdtype(t.dtype, jnp.floating) else t)(jnp.asarray(a)))
    def _A_setup():
        B, H, Sq, Sk, D, M = 1, 32, 1, 32768, 128, 512
        Dc = 4 * D
        return {
            "x": _w((lambda *s: _rng.normal(s) * 0.05)(B, Sq, M)),
            "c_kv": _w((lambda *s: _rng.normal(s) * 0.05)(B, Sk, Dc)),
            "w_q": _w((lambda *s: _rng.normal(s) * 0.05)(M, H, D) * (M ** -0.5)),
            "w_uk": _w((lambda *s: _rng.normal(s) * 0.05)(Dc, H, D) * (Dc ** -0.5)),
            "w_uv": _w((lambda *s: _rng.normal(s) * 0.05)(Dc, H, D) * (Dc ** -0.5)),
            "w_o": _w((lambda *s: _rng.normal(s) * 0.05)(H, D, M) * ((H * D) ** -0.5)),
        }
    _A_in = _A_setup()

    def _B_setup():
        B, S, D, F = 1, 1, 512, 1376
        return {
            "x": _w((lambda *s: _rng.normal(s) * 0.05)(B, S, D)),
            "w1": _w((lambda *s: _rng.normal(s) * 0.05)(D, F) * (D ** -0.5)),
            "w2": _w((lambda *s: _rng.normal(s) * 0.05)(F, D) * (F ** -0.5)),
        }
    _B_in = _B_setup()

    return {
        "A_x": _A_in["x"],
        "A_c_kv": _A_in["c_kv"],
        "A_w_q": _A_in["w_q"],
        "A_w_uk": _A_in["w_uk"],
        "A_w_uv": _A_in["w_uv"],
        "A_w_o": _A_in["w_o"],
        "B_x": _B_in["x"],
        "B_w1": _B_in["w1"],
        "B_w2": _B_in["w2"],
    }

def reference(A_x, A_c_kv, A_w_q, A_w_uk, A_w_uv, A_w_o, B_x, B_w1, B_w2):
    def _A_ref(x, c_kv, w_q, w_uk, w_uv, w_o):
        B, Sq, M = x.shape[0], x.shape[1], x.shape[2]
        Sk = c_kv.shape[1]
        H, D = w_q.shape[1], w_q.shape[2]
        q = jnp.einsum("bqm,mhd->bhqd", x, w_q)
        k = jnp.einsum("bkc,chd->bhkd", c_kv, w_uk)
        v = jnp.einsum("bkc,chd->bhkd", c_kv, w_uv)
        scores = jnp.einsum("bhqd,bhkd->bhqk", q, k) * (D ** -0.5)
        off = Sk - Sq
        qi = jnp.arange(Sq)[:, None]
        kj = jnp.arange(Sk)[None, :]
        cmask = kj <= (qi + off)
        scores = jnp.where(cmask[None, None], scores, -1e9)
        p = _softmax(scores, axis=-1)
        ctx = jnp.einsum("bhqk,bhkd->bhqd", p, v)
        return jnp.einsum("bhqd,hdm->bqm", ctx, w_o)

    def _B_ref(x, w1, w2):
        h = jnp.einsum("bsd,df->bsf", x, w1)
        h = _silu(h)
        out = jnp.einsum("bsf,fd->bsd", h, w2)
        return out

    x = A_x
    xn = _layernorm(x, axis=-1)
    s = _A_ref(xn, A_c_kv, A_w_q, A_w_uk, A_w_uv, A_w_o)
    g = _silu(_B_ref(xn, B_w1, B_w2))
    return x + s * g
```

```python
import jax
import jax.numpy as jnp
import numpy as np
from jax import lax
from jax.experimental import pallas as pl
from jax.experimental.pallas import tpu as pltpu

BF = jnp.bfloat16
F32 = jnp.float32
H, D, M, DC, SK, FF = 32, 128, 512, 512, 32768, 1376
LOG2E = 1.4426950408889634
NT = (((1,), (1,)), ((), ()))


def build(CH=2048, TK=512, WO_PIECES=(16, 8, 4, 4), UNROLL_T=8, sub_unroll=True, ffn_first=False):
  n_ch = SK // CH
  n_sub = CH // TK
  n_wo = len(WO_PIECES)
  wo_start = np.cumsum([0] + list(WO_PIECES))[:-1]

  def kernel(x_hbm, c_hbm, wq_hbm, wuk_hbm, wuv_hbm, wo_hbm, w1t_hbm, w2_hbm, o_ref,
             x_v, c_v, wq_v, wuk_v, wuv_v, wo_v, w1t_v, w2_v, y_v, lhs_v, csem, wsem):
    cp_x = pltpu.make_async_copy(x_hbm, x_v, wsem.at[0])
    cp_q = pltpu.make_async_copy(wq_hbm, wq_v, wsem.at[1])
    cp_uk = pltpu.make_async_copy(wuk_hbm, wuk_v, wsem.at[2])
    cp_w1 = pltpu.make_async_copy(w1t_hbm, w1t_v, wsem.at[3])
    cp_w2 = pltpu.make_async_copy(w2_hbm, w2_v, wsem.at[4])
    cp_uv = pltpu.make_async_copy(wuv_hbm, wuv_v, wsem.at[5])
    cp_o = [pltpu.make_async_copy(wo_hbm.at[pl.ds(int(s), n)], wo_v.at[pl.ds(int(s), n)], wsem.at[6 + i])
            for i, (s, n) in enumerate(zip(wo_start, WO_PIECES))]

    def cp_c(k):
      return pltpu.make_async_copy(c_hbm.at[0, pl.ds(k * CH, CH)], c_v.at[pl.ds(k * CH, CH)], csem.at[k])

    cp_x.start()
    cp_q.start()
    cp_uk.start()
    if ffn_first:
      cp_w1.start(); cp_w2.start()
    for k in range(n_ch):
      cp_c(k).start()
    if not ffn_first:
      cp_w1.start(); cp_w2.start()
    cp_uv.start()
    for c in cp_o:
      c.start()

    row32 = lax.broadcasted_iota(jnp.int32, (H, 128), 0)
    lane32 = lax.broadcasted_iota(jnp.int32, (H, 128), 1)
    diag = (lane32 % H) == row32

    cp_x.wait()
    xf = x_v[...].astype(F32)
    mu = jnp.mean(xf, axis=-1, keepdims=True)
    xc = xf - mu
    var = jnp.mean(xc * xc, axis=-1, keepdims=True)
    xn = xc / jnp.sqrt(var + 1e-5)

    def contract_major(coef, w_v):
      stack = jnp.concatenate([coef[:, 128 * u:128 * (u + 1)] for u in range(4)], axis=0)
      y_v[...] = stack.T

      def body(g, acc):
        a_parts, t_parts = [], []
        y8 = y_v[pl.ds(pl.multiple_of(g * UNROLL_T, UNROLL_T), UNROLL_T), :]
        for i in range(UNROLL_T):
          t = g * UNROLL_T + i
          rowt = jnp.broadcast_to(y8[i:i + 1, :], (H, 128))
          a_parts.append(jnp.where(diag, rowt, 0.0).astype(BF))
          for u in range(4):
            t_parts.append(w_v[128 * u + t])
        a = jnp.concatenate(a_parts, axis=1)
        tt = jnp.concatenate(t_parts, axis=0)
        return acc + jnp.dot(a, tt, preferred_element_type=F32)

      return lax.fori_loop(0, 128 // UNROLL_T, body, jnp.zeros((H, 128), F32))

    cp_q.wait()
    q = contract_major(jnp.broadcast_to(xn, (H, M)), wq_v)
    q_b = q.astype(BF)

    cp_uk.wait()

    def qp_body(g, _):
      t_parts = []
      for i in range(UNROLL_T):
        t = g * UNROLL_T + i
        for u in range(4):
          t_parts.append(wuk_v[128 * u + t])
      tt = jnp.concatenate(t_parts, axis=0)
      out = lax.dot_general(q_b, tt, NT, preferred_element_type=F32)
      rows = [jnp.sum(jnp.where(diag, out[:, 128 * i:128 * (i + 1)], 0.0), axis=0, keepdims=True)
              for i in range(UNROLL_T)]
      y_v[pl.ds(pl.multiple_of(g * UNROLL_T, UNROLL_T), UNROLL_T), :] = jnp.concatenate(rows, axis=0)
      return 0

    lax.fori_loop(0, 128 // UNROLL_T, qp_body, 0)
    zt = y_v[...].T
    qp = jnp.concatenate([zt[32 * u:32 * (u + 1), :] for u in range(4)], axis=1)
    qp_b = (qp * (D ** -0.5 * LOG2E)).astype(BF)

    def block(base, carry):
      m, l, acc = carry
      cb = c_v[pl.ds(base, TK), :]
      s = lax.dot_general(qp_b, cb, NT, preferred_element_type=F32)
      m_new = jnp.maximum(m, jnp.max(s, axis=-1, keepdims=True))
      alpha = jnp.exp2(m - m_new)
      p = jnp.exp2(s - m_new)
      ps = p[:, 0:128]
      for j in range(1, TK // 128):
        ps = ps + p[:, 128 * j:128 * (j + 1)]
      l = alpha * l + ps
      cb2 = c_v[pl.ds(base, TK), :]
      acc = alpha * acc + jnp.dot(p.astype(BF), cb2, preferred_element_type=F32)
      return m_new, l, acc

    def chunk(k, carry):
      cp_c(k).wait()
      if sub_unroll:
        for j in range(n_sub):
          carry = block(pl.multiple_of(k * CH + j * TK, TK), carry)
        return carry
      return lax.fori_loop(0, n_sub, lambda j, c: block(pl.multiple_of(k * CH + j * TK, TK), c), carry)

    init = (jnp.full((H, 1), -1e30, F32), jnp.zeros((H, 128), F32), jnp.zeros((H, DC), F32))
    m, l, acc = lax.fori_loop(0, n_ch, chunk, init)
    cc = acc / jnp.sum(l, axis=-1, keepdims=True)

    xn16 = jnp.broadcast_to(xn, (16, M)).astype(BF)
    cp_w1.wait()
    h1 = lax.dot_general(xn16, w1t_v[...], NT, preferred_element_type=F32)
    h1 = h1 * jax.nn.sigmoid(h1)
    cp_w2.wait()
    o2 = jnp.dot(h1.astype(BF), w2_v[...], preferred_element_type=F32)
    g = o2 * jax.nn.sigmoid(o2)

    cp_uv.wait()
    ctx = contract_major(cc, wuv_v)
    for h in range(H):
      lhs_v[:, 128 * h:128 * (h + 1)] = jnp.broadcast_to(ctx[h:h + 1, :], (16, 128)).astype(BF)

    sacc = jnp.zeros((16, M), F32)
    for i, (s0, n) in enumerate(zip(wo_start, WO_PIECES)):
      s0 = int(s0)
      cp_o[i].wait()
      w = wo_v[pl.ds(s0, n)].reshape(n * 128, M)
      sacc = sacc + jnp.dot(lhs_v[:, 128 * s0:128 * (s0 + n)], w, preferred_element_type=F32)
    y = xf + sacc[0:1, :] * g[0:1, :]
    o_ref[...] = y.astype(BF)

  def f(A_x, A_c_kv, A_w_q, A_w_uk, A_w_uv, A_w_o, B_x, B_w1, B_w2):
    anyspec = pl.BlockSpec(memory_space=pl.ANY)
    out = pl.pallas_call(
        kernel,
        out_shape=jax.ShapeDtypeStruct((1, M), BF),
        in_specs=[anyspec] * 8,
        out_specs=pl.BlockSpec(memory_space=pltpu.VMEM),
        scratch_shapes=[
            pltpu.VMEM((1, M), BF), pltpu.VMEM((SK, DC), BF),
            pltpu.VMEM((M, H, D), BF), pltpu.VMEM((DC, H, D), BF), pltpu.VMEM((DC, H, D), BF),
            pltpu.VMEM((H, D, M), BF), pltpu.VMEM((FF, M), BF), pltpu.VMEM((FF, M), BF),
            pltpu.VMEM((128, 128), F32), pltpu.VMEM((16, H * D), BF),
            pltpu.SemaphoreType.DMA((n_ch,)), pltpu.SemaphoreType.DMA((6 + n_wo,))],
        compiler_params=pltpu.CompilerParams(vmem_limit_bytes=100 * 1024 * 1024),
        name="mla_decode",
    )(A_x.reshape(1, M), A_c_kv, A_w_q, A_w_uk, A_w_uv, A_w_o, B_w1.T, B_w2)
    return out.reshape(1, 1, M)
  return jax.jit(f)


_kernel = build(TK=1024)


@jax.jit
def pallas_recurrent_scan__compressed_kv_cla__dense_activation_silu__decode_kernel(
    A_x, A_c_kv, A_w_q, A_w_uk, A_w_uv, A_w_o, B_x, B_w1, B_w2):
  return _kernel(A_x, A_c_kv, A_w_q, A_w_uk, A_w_uv, A_w_o, B_x, B_w1, B_w2)
```

```python
import jax
import jax.numpy as jnp
import numpy as np
from jax import lax
from jax.experimental import pallas as pl
from jax.experimental.pallas import tpu as pltpu

BF = jnp.bfloat16
F32 = jnp.float32
H, D, M, DC, SK, FF = 32, 128, 512, 512, 32768, 1376
LOG2E = 1.4426950408889634
NT = (((1,), (1,)), ((), ()))


def build(C_PIECES=(16384, 8192, 8192), TK=1024, WO_PIECES=(28, 4), UNROLL_T=8, G=4, skip=()):
  assert sum(C_PIECES) == SK and all(p % TK == 0 for p in C_PIECES) and sum(WO_PIECES) == H and all(p % G == 0 for p in WO_PIECES)
  n_c, n_wo = len(C_PIECES), len(WO_PIECES)
  c_start = [int(v) for v in np.cumsum((0,) + tuple(C_PIECES))[:-1]]
  wo_start = [int(v) for v in np.cumsum((0,) + tuple(WO_PIECES))[:-1]]

  def kernel(x_hbm, c_hbm, wq_hbm, wuk_hbm, wuv_hbm, wo_hbm, w1t_hbm, w2_hbm, o_ref,
             x_v, c_v, wq_v, wuk_v, wuv_v, wo_v, w1t_v, w2_v, y_v, lhs_v, sem):
    srcdst = [(x_hbm, x_v), (w1t_hbm, w1t_v), (w2_hbm, w2_v), (wq_hbm, wq_v), (wuk_hbm, wuk_v)]
    srcdst += [(c_hbm.at[0, pl.ds(s, n)], c_v.at[pl.ds(s, n)]) for s, n in zip(c_start, C_PIECES)]
    srcdst += [(wuv_hbm, wuv_v)]
    srcdst += [(wo_hbm.at[pl.ds(s, n)], wo_v.at[pl.ds(s, n)]) for s, n in zip(wo_start, WO_PIECES)]
    cps = [pltpu.make_async_copy(s, d, sem.at[i]) for i, (s, d) in enumerate(srcdst)]
    cp_x, cp_w1, cp_w2, cp_q, cp_uk = cps[:5]
    cp_c = cps[5:5 + n_c]
    cp_uv = cps[5 + n_c]
    cp_o = cps[6 + n_c:]
    for c in cps:
      c.start()

    row32 = lax.broadcasted_iota(jnp.int32, (H, 128), 0)
    lane32 = lax.broadcasted_iota(jnp.int32, (H, 128), 1)
    diag = (lane32 % H) == row32

    cp_x.wait()
    xf = x_v[...].astype(F32)
    mu = jnp.mean(xf, axis=-1, keepdims=True)
    xc = xf - mu
    var = jnp.mean(xc * xc, axis=-1, keepdims=True)
    xn = xc / jnp.sqrt(var + 1e-5)

    xn16 = jnp.broadcast_to(xn, (16, M)).astype(BF)
    cp_w1.wait()
    h1 = lax.dot_general(xn16, w1t_v[...], NT, preferred_element_type=F32)
    h1 = h1 * jax.nn.sigmoid(h1)
    cp_w2.wait()
    o2 = jnp.dot(h1.astype(BF), w2_v[...], preferred_element_type=F32)
    g = o2 * jax.nn.sigmoid(o2)

    def gather_tiles(w_v, g):
      return jnp.concatenate([w_v[128 * u + g * UNROLL_T + i] for i in range(UNROLL_T) for u in range(4)], axis=0)

    def contract_major(coef, w_v):
      stack = jnp.concatenate([coef[:, 128 * u:128 * (u + 1)] for u in range(4)], axis=0)
      y_v[...] = stack.T

      def body(g, acc):
        y8 = y_v[pl.ds(pl.multiple_of(g * UNROLL_T, UNROLL_T), UNROLL_T), :]
        a = jnp.concatenate(
            [jnp.where(diag, jnp.broadcast_to(y8[i:i + 1, :], (H, 128)), 0.0).astype(BF) for i in range(UNROLL_T)],
            axis=1)
        return acc + jnp.dot(a, gather_tiles(w_v, g), preferred_element_type=F32)

      return lax.fori_loop(0, 128 // UNROLL_T, body, jnp.zeros((H, 128), F32))

    cp_q.wait()
    q_b = contract_major(jnp.broadcast_to(xn, (H, M)), wq_v).astype(BF)

    cp_uk.wait()

    def qp_body(g, _):
      out = lax.dot_general(q_b, gather_tiles(wuk_v, g), NT, preferred_element_type=F32)
      rows = [jnp.sum(jnp.where(diag, out[:, 128 * i:128 * (i + 1)], 0.0), axis=0, keepdims=True)
              for i in range(UNROLL_T)]
      y_v[pl.ds(pl.multiple_of(g * UNROLL_T, UNROLL_T), UNROLL_T), :] = jnp.concatenate(rows, axis=0)
      return 0

    lax.fori_loop(0, 128 // UNROLL_T, qp_body, 0)
    zt = y_v[...].T
    qp = jnp.concatenate([zt[32 * u:32 * (u + 1), :] for u in range(4)], axis=1)
    qp_b = (qp * (D ** -0.5 * LOG2E)).astype(BF)

    def block(b, carry):
      for cp, s0 in zip(cp_c, c_start):
        @pl.when(b == s0 // TK)
        def _():
          cp.wait()
      if 'main' in skip:
        return carry
      m, l, acc = carry
      base = pl.multiple_of(b * TK, TK)
      s = lax.dot_general(qp_b, c_v[pl.ds(base, TK), :], NT, preferred_element_type=F32)
      m_new = jnp.maximum(m, jnp.max(s, axis=-1, keepdims=True))
      alpha = jnp.exp2(m - m_new)
      p = jnp.exp2(s - m_new)
      ps = p[:, 0:128]
      for j in range(1, TK // 128):
        ps = ps + p[:, 128 * j:128 * (j + 1)]
      l = alpha * l + ps
      acc = alpha * acc + jnp.dot(p.astype(BF), c_v[pl.ds(base, TK), :], preferred_element_type=F32)
      return m_new, l, acc

    init = (jnp.full((H, 1), -1e30, F32), jnp.zeros((H, 128), F32), jnp.zeros((H, DC), F32))
    m, l, acc = lax.fori_loop(0, SK // TK, block, init)
    cc = acc / jnp.sum(l, axis=-1, keepdims=True)

    cp_uv.wait()
    ctx = contract_major(cc, wuv_v)
    for h in range(H):
      lhs_v[h] = jnp.broadcast_to(ctx[h:h + 1, :], (16, 128)).astype(BF)

    def wo_body(i, sacc):
      for cp, s0 in zip(cp_o, wo_start):
        @pl.when(i == s0 // G)
        def _():
          cp.wait()
      a = jnp.concatenate([lhs_v[i * G + j] for j in range(G)], axis=1)
      w = wo_v[pl.ds(i * G, G)].reshape(G * 128, M)
      return sacc + jnp.dot(a, w, preferred_element_type=F32)

    sacc = lax.fori_loop(0, H // G, wo_body, jnp.zeros((16, M), F32))
    y = xf + sacc[0:1, :] * g[0:1, :]
    o_ref[...] = y.astype(BF)

  def f(A_x, A_c_kv, A_w_q, A_w_uk, A_w_uv, A_w_o, B_x, B_w1, B_w2):
    anyspec = pl.BlockSpec(memory_space=pl.ANY)
    out = pl.pallas_call(
        kernel,
        out_shape=jax.ShapeDtypeStruct((1, M), BF),
        in_specs=[anyspec] * 8,
        out_specs=pl.BlockSpec(memory_space=pltpu.VMEM),
        scratch_shapes=[
            pltpu.VMEM((1, M), BF), pltpu.VMEM((SK, DC), BF),
            pltpu.VMEM((M, H, D), BF), pltpu.VMEM((DC, H, D), BF), pltpu.VMEM((DC, H, D), BF),
            pltpu.VMEM((H, D, M), BF), pltpu.VMEM((FF, M), BF), pltpu.VMEM((FF, M), BF),
            pltpu.VMEM((128, 128), F32), pltpu.VMEM((H, 16, D), BF),
            pltpu.SemaphoreType.DMA((6 + n_c + n_wo,))],
        compiler_params=pltpu.CompilerParams(vmem_limit_bytes=100 * 1024 * 1024),
        name="mla_decode",
    )(A_x.reshape(1, M), A_c_kv, A_w_q, A_w_uk, A_w_uv, A_w_o, B_w1.T, B_w2)
    return out.reshape(1, 1, M)
  return jax.jit(f)


_kernel = build(C_PIECES=(16384, 8192, 8192), WO_PIECES=(20, 8, 4), TK=1024, G=4)


@jax.jit
def pallas_recurrent_scan__compressed_kv_cla__dense_activation_silu__decode_kernel(
    A_x, A_c_kv, A_w_q, A_w_uk, A_w_uv, A_w_o, B_x, B_w1, B_w2):
  return _kernel(A_x, A_c_kv, A_w_q, A_w_uk, A_w_uv, A_w_o, B_x, B_w1, B_w2)
```

```python
import jax
import jax.numpy as jnp
import numpy as np
from jax import lax
from jax.experimental import pallas as pl
from jax.experimental.pallas import tpu as pltpu

BF = jnp.bfloat16
F32 = jnp.float32

H, D, M, DC, SK, FF = 32, 128, 512, 512, 32768, 1376
LOG2E = 1.4426950408889634
NT = (((1,), (1,)), ((), ()))

C_PIECES = (16384, 10240, 6144)
WO_PIECES = (20, 8, 4)
TK = 2048
UT = 8
G = 4

_C_START = tuple(int(v) for v in np.cumsum((0,) + C_PIECES)[:-1])
_WO_START = tuple(int(v) for v in np.cumsum((0,) + WO_PIECES)[:-1])


def _kernel(x_hbm, c_hbm, wq_hbm, wuk_hbm, wuv_hbm, wo_hbm, w1t_hbm, w2_hbm, o_ref,
            x_v, c_v, wq_v, wuk_v, wuv_v, wo_v, w1t_v, w2_v, y_v, lhs_v, sem):
  pairs = [(x_hbm, x_v), (w1t_hbm, w1t_v), (w2_hbm, w2_v), (wq_hbm, wq_v), (wuk_hbm, wuk_v)]
  pairs += [(c_hbm.at[0, pl.ds(s, n)], c_v.at[pl.ds(s, n)]) for s, n in zip(_C_START, C_PIECES)]
  pairs += [(wuv_hbm, wuv_v)]
  pairs += [(wo_hbm.at[pl.ds(s, n)], wo_v.at[pl.ds(s, n)]) for s, n in zip(_WO_START, WO_PIECES)]
  copies = [pltpu.make_async_copy(src, dst, sem.at[i]) for i, (src, dst) in enumerate(pairs)]
  cp_x, cp_w1, cp_w2, cp_q, cp_uk = copies[:5]
  cp_c = copies[5:5 + len(C_PIECES)]
  cp_uv = copies[5 + len(C_PIECES)]
  cp_o = copies[6 + len(C_PIECES):]
  for cp in copies:
    cp.start()

  row = lax.broadcasted_iota(jnp.int32, (H, 128), 0)
  lane = lax.broadcasted_iota(jnp.int32, (H, 128), 1)
  diag = (lane % H) == row

  def tiles(w_v, g):
    return jnp.concatenate(
        [w_v[128 * u + g * UT + i] for i in range(UT) for u in range(4)], axis=0)

  def contract_major(coef, w_v):
    stack = jnp.concatenate([coef[:, 128 * u:128 * (u + 1)] for u in range(4)], axis=0)
    y_v[...] = stack.T

    def body(g, acc):
      y = y_v[pl.ds(pl.multiple_of(g * UT, UT), UT), :]
      a = jnp.concatenate(
          [jnp.where(diag, jnp.broadcast_to(y[i:i + 1, :], (H, 128)), 0.0).astype(BF)
           for i in range(UT)], axis=1)
      return acc + jnp.dot(a, tiles(w_v, g), preferred_element_type=F32)

    return lax.fori_loop(0, 128 // UT, body, jnp.zeros((H, D), F32))

  cp_x.wait()
  xf = x_v[...].astype(F32)
  xc = xf - jnp.mean(xf, axis=-1, keepdims=True)
  xn = xc / jnp.sqrt(jnp.mean(xc * xc, axis=-1, keepdims=True) + 1e-5)

  xn16 = jnp.broadcast_to(xn, (16, M)).astype(BF)
  cp_w1.wait()
  h1 = lax.dot_general(xn16, w1t_v[...], NT, preferred_element_type=F32)
  h1 = h1 * jax.nn.sigmoid(h1)
  cp_w2.wait()
  o2 = jnp.dot(h1.astype(BF), w2_v[...], preferred_element_type=F32)
  gate = o2 * jax.nn.sigmoid(o2)

  cp_q.wait()
  q = contract_major(jnp.broadcast_to(xn, (H, M)), wq_v).astype(BF)

  cp_uk.wait()

  def qa_body(g, carry):
    out = lax.dot_general(q, tiles(wuk_v, g), NT, preferred_element_type=F32)
    y_v[pl.ds(pl.multiple_of(g * UT, UT), UT), :] = jnp.concatenate(
        [jnp.sum(jnp.where(diag, out[:, 128 * i:128 * (i + 1)], 0.0), axis=0, keepdims=True)
         for i in range(UT)], axis=0)
    return carry

  lax.fori_loop(0, 128 // UT, qa_body, 0)
  zt = y_v[...].T
  qa = jnp.concatenate([zt[H * u:H * (u + 1), :] for u in range(4)], axis=1)
  qa = (qa * (D ** -0.5 * LOG2E)).astype(BF)

  def block(b, carry):
    for cp, s0 in zip(cp_c, _C_START):
      @pl.when(b == s0 // TK)
      def _():
        cp.wait()
    m, l, acc = carry
    keys = pl.ds(pl.multiple_of(b * TK, TK), TK)
    s = lax.dot_general(qa, c_v[keys, :], NT, preferred_element_type=F32)
    m_new = jnp.maximum(m, jnp.max(s, axis=-1, keepdims=True))
    alpha = jnp.exp2(m - m_new)
    p = jnp.exp2(s - m_new)
    psum = p[:, 0:128]
    for j in range(1, TK // 128):
      psum = psum + p[:, 128 * j:128 * (j + 1)]
    l = alpha * l + psum
    acc = alpha * acc + jnp.dot(p.astype(BF), c_v[keys, :], preferred_element_type=F32)
    return m_new, l, acc

  init = (jnp.full((H, 1), -1e30, F32), jnp.zeros((H, 128), F32), jnp.zeros((H, DC), F32))
  _, l, acc = lax.fori_loop(0, SK // TK, block, init)
  cc = acc / jnp.sum(l, axis=-1, keepdims=True)

  cp_uv.wait()
  ctx = contract_major(cc, wuv_v)
  for h in range(H):
    lhs_v[h] = jnp.broadcast_to(ctx[h:h + 1, :], (16, D)).astype(BF)

  def wo_body(i, s_acc):
    for cp, s0 in zip(cp_o, _WO_START):
      @pl.when(i == s0 // G)
      def _():
        cp.wait()
    a = jnp.concatenate([lhs_v[i * G + j] for j in range(G)], axis=1)
    w = wo_v[pl.ds(i * G, G)].reshape(G * D, M)
    return s_acc + jnp.dot(a, w, preferred_element_type=F32)

  s_out = lax.fori_loop(0, H // G, wo_body, jnp.zeros((16, M), F32))
  o_ref[...] = (xf + s_out[0:1, :] * gate[0:1, :]).astype(o_ref.dtype)


@jax.jit
def pallas_recurrent_scan__compressed_kv_cla__dense_activation_silu__decode_kernel(
    A_x: jax.Array,
    A_c_kv: jax.Array,
    A_w_q: jax.Array,
    A_w_uk: jax.Array,
    A_w_uv: jax.Array,
    A_w_o: jax.Array,
    B_x: jax.Array,
    B_w1: jax.Array,
    B_w2: jax.Array,
):
  del B_x
  hbm = pl.BlockSpec(memory_space=pl.ANY)
  n_copies = 6 + len(C_PIECES) + len(WO_PIECES)
  out = pl.pallas_call(
      _kernel,
      out_shape=jax.ShapeDtypeStruct((1, M), A_x.dtype),
      in_specs=[hbm] * 8,
      out_specs=pl.BlockSpec(memory_space=pltpu.VMEM),
      scratch_shapes=[
          pltpu.VMEM((1, M), BF),
          pltpu.VMEM((SK, DC), BF),
          pltpu.VMEM((M, H, D), BF),
          pltpu.VMEM((DC, H, D), BF),
          pltpu.VMEM((DC, H, D), BF),
          pltpu.VMEM((H, D, M), BF),
          pltpu.VMEM((FF, M), BF),
          pltpu.VMEM((FF, M), BF),
          pltpu.VMEM((128, 128), F32),
          pltpu.VMEM((H, 16, D), BF),
          pltpu.SemaphoreType.DMA((n_copies,)),
      ],
      compiler_params=pltpu.CompilerParams(vmem_limit_bytes=100 * 1024 * 1024),
      name="mla_decode_silu_gate",
  )(
      A_x.reshape(1, M), A_c_kv, A_w_q, A_w_uk, A_w_uv, A_w_o,
      B_w1.T,
      B_w2,
  )
  return out.reshape(1, 1, M)
```

```python
import jax
import jax.numpy as jnp
import numpy as np
from jax import lax
from jax.experimental import pallas as pl
from jax.experimental.pallas import tpu as pltpu

BF = jnp.bfloat16
F32 = jnp.float32

H, D, M, DC, SK, FF = 32, 128, 512, 512, 32768, 1376
LOG2E = 1.4426950408889634
NT = (((1,), (1,)), ((), ()))

C_PIECES = (12288, 10240, 6144, 4096)
WO_PIECES = (20, 8, 4)
TK = 2048
UT = 8
G = 4

_C_START = tuple(int(v) for v in np.cumsum((0,) + C_PIECES)[:-1])
_WO_START = tuple(int(v) for v in np.cumsum((0,) + WO_PIECES)[:-1])


def _kernel(x_hbm, c_hbm, wq_hbm, wuk_hbm, wuv_hbm, wo_hbm, w1t_hbm, w2_hbm, o_ref,
            x_v, c_v, wq_v, wuk_v, wuv_v, wo_v, w1t_v, w2_v, y_v, lhs_v, sem):
  pairs = [(x_hbm, x_v), (w1t_hbm, w1t_v), (w2_hbm, w2_v), (wq_hbm, wq_v), (wuk_hbm, wuk_v)]
  pairs += [(c_hbm.at[0, pl.ds(s, n)], c_v.at[pl.ds(s, n)]) for s, n in zip(_C_START, C_PIECES)]
  pairs += [(wuv_hbm, wuv_v)]
  pairs += [(wo_hbm.at[pl.ds(s, n)], wo_v.at[pl.ds(s, n)]) for s, n in zip(_WO_START, WO_PIECES)]
  copies = [pltpu.make_async_copy(src, dst, sem.at[i]) for i, (src, dst) in enumerate(pairs)]
  cp_x, cp_w1, cp_w2, cp_q, cp_uk = copies[:5]
  cp_c = copies[5:5 + len(C_PIECES)]
  cp_uv = copies[5 + len(C_PIECES)]
  cp_o = copies[6 + len(C_PIECES):]
  for cp in copies:
    cp.start()

  row = lax.broadcasted_iota(jnp.int32, (H, 128), 0)
  lane = lax.broadcasted_iota(jnp.int32, (H, 128), 1)
  diag = (lane % H) == row

  def hilo(v):
    hi = v.astype(BF)
    return jnp.concatenate([hi, (v - hi.astype(F32)).astype(BF)], axis=0)

  def tiles(w_v, g):
    return jnp.concatenate(
        [w_v[128 * u + g * UT + i] for i in range(UT) for u in range(4)], axis=0)

  def contract_major(coef, w_v, split):
    to_mxu = hilo if split else (lambda v: v.astype(BF))
    stack = jnp.concatenate([coef[:, 128 * u:128 * (u + 1)] for u in range(4)], axis=0)
    y_v[...] = stack.T

    def body(g, acc):
      y = y_v[pl.ds(pl.multiple_of(g * UT, UT), UT), :]
      a = jnp.concatenate(
          [to_mxu(jnp.where(diag, jnp.broadcast_to(y[i:i + 1, :], (H, 128)), 0.0))
           for i in range(UT)], axis=1)
      return acc + jnp.dot(a, tiles(w_v, g), preferred_element_type=F32)

    out = lax.fori_loop(0, 128 // UT, body, jnp.zeros((2 * H if split else H, D), F32))
    return out[:H] + out[H:] if split else out

  cp_x.wait()
  xf = x_v[...].astype(F32)
  xc = xf - jnp.mean(xf, axis=-1, keepdims=True)
  xn = xc / jnp.sqrt(jnp.mean(xc * xc, axis=-1, keepdims=True) + 1e-5)

  xn16 = jnp.broadcast_to(xn, (16, M)).astype(BF)
  cp_w1.wait()
  h1 = lax.dot_general(xn16, w1t_v[...], NT, preferred_element_type=F32)
  h1 = h1 * jax.nn.sigmoid(h1)
  cp_w2.wait()
  o2 = jnp.dot(h1.astype(BF), w2_v[...], preferred_element_type=F32)
  gate = o2 * jax.nn.sigmoid(o2)

  cp_q.wait()
  q = hilo(contract_major(jnp.broadcast_to(xn, (H, M)), wq_v, split=True))

  cp_uk.wait()

  def qa_body(g, carry):
    out = lax.dot_general(q, tiles(wuk_v, g), NT, preferred_element_type=F32)
    out = out[:H] + out[H:]
    y_v[pl.ds(pl.multiple_of(g * UT, UT), UT), :] = jnp.concatenate(
        [jnp.sum(jnp.where(diag, out[:, 128 * i:128 * (i + 1)], 0.0), axis=0, keepdims=True)
         for i in range(UT)], axis=0)
    return carry

  lax.fori_loop(0, 128 // UT, qa_body, 0)
  zt = y_v[...].T
  qa = jnp.concatenate([zt[H * u:H * (u + 1), :] for u in range(4)], axis=1)
  qa = hilo(qa * (D ** -0.5 * LOG2E))

  def block(b, carry):
    for cp, s0 in zip(cp_c, _C_START):
      @pl.when(b == s0 // TK)
      def _():
        cp.wait()
    m, l, acc = carry
    keys = pl.ds(pl.multiple_of(b * TK, TK), TK)
    s = lax.dot_general(qa, c_v[keys, :], NT, preferred_element_type=F32)
    s = s[:H] + s[H:]
    m_new = jnp.maximum(m, jnp.max(s, axis=-1, keepdims=True))
    alpha = jnp.exp2(m - m_new)
    p = jnp.exp2(s - m_new)
    psum = p[:, 0:128]
    for j in range(1, TK // 128):
      psum = psum + p[:, 128 * j:128 * (j + 1)]
    l = alpha * l + psum
    acc = alpha * acc + jnp.dot(p.astype(BF), c_v[keys, :], preferred_element_type=F32)
    return m_new, l, acc

  init = (jnp.full((H, 1), -1e30, F32), jnp.zeros((H, 128), F32), jnp.zeros((H, DC), F32))
  _, l, acc = lax.fori_loop(0, SK // TK, block, init)
  cc = acc / jnp.sum(l, axis=-1, keepdims=True)

  cp_uv.wait()
  ctx = contract_major(cc, wuv_v, split=False)
  for h in range(H):
    lhs_v[h] = jnp.broadcast_to(ctx[h:h + 1, :], (16, D)).astype(BF)

  def wo_body(i, s_acc):
    for cp, s0 in zip(cp_o, _WO_START):
      @pl.when(i == s0 // G)
      def _():
        cp.wait()
    a = jnp.concatenate([lhs_v[i * G + j] for j in range(G)], axis=1)
    w = wo_v[pl.ds(i * G, G)].reshape(G * D, M)
    return s_acc + jnp.dot(a, w, preferred_element_type=F32)

  s_out = lax.fori_loop(0, H // G, wo_body, jnp.zeros((16, M), F32))
  o_ref[...] = (xf + s_out[0:1, :] * gate[0:1, :]).astype(o_ref.dtype)


@jax.jit
def pallas_recurrent_scan__compressed_kv_cla__dense_activation_silu__decode_kernel(
    A_x: jax.Array,
    A_c_kv: jax.Array,
    A_w_q: jax.Array,
    A_w_uk: jax.Array,
    A_w_uv: jax.Array,
    A_w_o: jax.Array,
    B_x: jax.Array,
    B_w1: jax.Array,
    B_w2: jax.Array,
):
  del B_x
  hbm = pl.BlockSpec(memory_space=pl.ANY)
  n_copies = 6 + len(C_PIECES) + len(WO_PIECES)
  out = pl.pallas_call(
      _kernel,
      out_shape=jax.ShapeDtypeStruct((1, M), A_x.dtype),
      in_specs=[hbm] * 8,
      out_specs=pl.BlockSpec(memory_space=pltpu.VMEM),
      scratch_shapes=[
          pltpu.VMEM((1, M), BF),
          pltpu.VMEM((SK, DC), BF),
          pltpu.VMEM((M, H, D), BF),
          pltpu.VMEM((DC, H, D), BF),
          pltpu.VMEM((DC, H, D), BF),
          pltpu.VMEM((H, D, M), BF),
          pltpu.VMEM((FF, M), BF),
          pltpu.VMEM((FF, M), BF),
          pltpu.VMEM((128, 128), F32),
          pltpu.VMEM((H, 16, D), BF),
          pltpu.SemaphoreType.DMA((n_copies,)),
      ],
      compiler_params=pltpu.CompilerParams(vmem_limit_bytes=100 * 1024 * 1024),
      name="mla_decode_silu_gate",
  )(
      A_x.reshape(1, M), A_c_kv, A_w_q, A_w_uk, A_w_uv, A_w_o,
      B_w1.T,
      B_w2,
  )
  return out.reshape(1, 1, M)
```
